```python
import jax
import jax.numpy as jnp

def _softmax(x, axis=-1):
    return jax.nn.softmax(x, axis=axis)

def _gelu(x):
    return jax.nn.gelu(x, approximate=True)

def _silu(x):
    return jax.nn.silu(x)

def _sigmoid(x):
    return jax.nn.sigmoid(x)

def _layernorm(x, axis=-1, eps=1e-05):
    m = jnp.mean(x, axis=axis, keepdims=True)
    v = jnp.var(x, axis=axis, keepdims=True)
    return (x - m) / jnp.sqrt(v + eps)

def _scatter_add(tgt, idx, src, axis=0):
    return tgt.at[idx].add(src)

def _segment_sum(src, seg, n):
    return jax.ops.segment_sum(src, seg, n)

class _Rng:

    def __init__(self, key):
        self._k = key

    def _next(self):
        self._k, sub = jax.random.split(self._k)
        return sub

    def normal(self, shape):
        return jax.random.normal(self._next(), shape, dtype=jnp.bfloat16)

    def randint(self, lo, hi, shape):
        return jax.random.randint(self._next(), shape, lo, hi, dtype=jnp.int32)

    def uniform(self, shape, lo=0.0, hi=1.0):
        return jax.random.uniform(self._next(), shape, jnp.bfloat16, lo, hi)

    def permutation(self, n):
        return jax.random.permutation(self._next(), n)
kernel_name = 'recurrent_scan__memory_aug_recurrent_mem_tr__glu_gated_glu__prompt'

def setup_inputs():
    _rng = _Rng(jax.random.key(int.from_bytes(__import__("os").urandom(4), "little")))
    _w = lambda a: (lambda t: t.astype(jnp.bfloat16) if jnp.issubdtype(t.dtype, jnp.floating) else t)(jnp.asarray(a))

    def _A_setup():
        B, S, Dm = (1, 2048, 1024)
        H, Dh = (32, 128)
        M, seg = (8, 32)
        seg = min(seg, S)
        S = S // seg * seg
        return {'x': _w((lambda *s: _rng.normal(s) * 0.05)(B, S, Dm)), 'mem0': _w((lambda *s: _rng.normal(s) * 0.05)(B, M, Dm)), 'Wq': _w((lambda *s: _rng.normal(s) * 0.05)(Dm, H, Dh) * Dm ** (-0.5)), 'Wk': _w((lambda *s: _rng.normal(s) * 0.05)(Dm, H, Dh) * Dm ** (-0.5)), 'Wv': _w((lambda *s: _rng.normal(s) * 0.05)(Dm, H, Dh) * Dm ** (-0.5)), 'Wo': _w((lambda *s: _rng.normal(s) * 0.05)(H, Dh, Dm) * (H * Dh) ** (-0.5)), 'seg_len': seg}
    _A_in = _A_setup()

    def _B_setup():
        B, S, D, F = (1, 2048, 1024, 3584)
        return {'x': _w((lambda *s: _rng.normal(s) * 0.05)(B, S, D)), 'w_gate': _w((lambda *s: _rng.normal(s) * 0.05)(D, F)), 'w_up': _w((lambda *s: _rng.normal(s) * 0.05)(D, F)), 'w_down': _w((lambda *s: _rng.normal(s) * 0.05)(F, D))}
    _B_in = _B_setup()
    return {'A_x': _A_in['x'], 'A_mem0': _A_in['mem0'], 'A_Wq': _A_in['Wq'], 'A_Wk': _A_in['Wk'], 'A_Wv': _A_in['Wv'], 'A_Wo': _A_in['Wo'], 'A_seg_len': _A_in['seg_len'], 'B_x': _B_in['x'], 'B_w_gate': _B_in['w_gate'], 'B_w_up': _B_in['w_up'], 'B_w_down': _B_in['w_down']}

def reference(A_x, A_mem0, A_Wq, A_Wk, A_Wv, A_Wo, A_seg_len, B_x, B_w_gate, B_w_up, B_w_down):

    def _A_ref(x, mem0, Wq, Wk, Wv, Wo, seg_len):
        B, S, Dm = x.shape
        H, Dh = (Wq.shape[1], Wq.shape[2])
        M = mem0.shape[1]
        scale = Dh ** (-0.5)
        n_seg = S // seg_len
        L = M + seg_len
        idx = jnp.arange(L)
        mask = (idx[:, None] < M) | (idx[:, None] >= idx[None, :])
        mem = mem0
        outs = []
        for s in range(n_seg):
            xs = x[:, s * seg_len:(s + 1) * seg_len, :].copy()
            h = jnp.concatenate([mem, xs], axis=1)
            q = jnp.einsum('btd,dhe->bhte', h, Wq)
            k = jnp.einsum('btd,dhe->bhte', h, Wk)
            v = jnp.einsum('btd,dhe->bhte', h, Wv)
            scores = jnp.einsum('bhqe,bhke->bhqk', q, k) * scale
            scores = jnp.where(mask[None, None], scores, -1000000000.0)
            p = _softmax(scores, axis=-1)
            o = jnp.einsum('bhqk,bhke->bhqe', p, v)
            o = jnp.einsum('bhte,hed->btd', o, Wo)
            mem = o[:, :M, :].copy()
            outs.append(o[:, M:, :])
        return jnp.concatenate(outs, axis=1)

    def _B_ref(x, w_gate, w_up, w_down):
        g = jnp.einsum('bsd,df->bsf', x, w_gate)
        u = jnp.einsum('bsd,df->bsf', x, w_up)
        h = _sigmoid(g) * u
        return jnp.einsum('bsf,fd->bsd', h, w_down)
    x = A_x
    xn = _layernorm(x, axis=-1)
    s = _A_ref(xn, A_mem0, A_Wq, A_Wk, A_Wv, A_Wo, A_seg_len)
    g = _silu(_B_ref(xn, B_w_gate, B_w_up, B_w_down))
    return x + s * g
```

```python
import functools

import jax
import jax.numpy as jnp
import jax.experimental.pallas as pl
import jax.experimental.pallas.tpu as pltpu

_PRE = 512
_FCH = 512


def _sigmoid(x):
    return 1.0 / (1.0 + jnp.exp(-x))


def _bf16(x):
    return x.astype(jnp.bfloat16)


def _w(ref_val):
    return pltpu.bitcast(ref_val, jnp.bfloat16)


def _dot(a, b):
    return jnp.dot(a, b, preferred_element_type=jnp.float32)


def _kernel(x_ref, mem0_ref, wq_hbm, wk_hbm, wv_hbm, wo_hbm, wg_hbm, wu_hbm, wd_hbm,
            out_ref,
            wqkv, wo, wg, wu, wd, stg, xn_scr, g_scr, acc_scr, cq, ck, cv, co, oa, ob,
            sem_glu, sem_qkv, sem_o,
            *, S, D, H, M, SEG, F):
    NF = F // 128
    ND = D // 128
    NCH = F // _FCH
    TPC = _FCH // 128
    scale = 128 ** (-0.5)

    def glu_copies(f):
        cps = []
        for j in range(TPC):
            c = f * TPC + j
            cps.append(pltpu.make_async_copy(
                wg_hbm.at[:, pl.ds(c * 128, 128)], wg.at[c].bitcast(jnp.bfloat16), sem_glu.at[f]))
            cps.append(pltpu.make_async_copy(
                wu_hbm.at[:, pl.ds(c * 128, 128)], wu.at[c].bitcast(jnp.bfloat16), sem_glu.at[f]))
        for n in range(ND):
            cps.append(pltpu.make_async_copy(
                wd_hbm.at[pl.ds(f * _FCH, _FCH), pl.ds(n * 128, 128)],
                wd.at[n, pl.ds(f * (_FCH // 2), _FCH // 2), :].bitcast(jnp.bfloat16), sem_glu.at[f]))
        return cps

    def qkv_copy(i, hbm):
        return pltpu.make_async_copy(hbm, stg.at[i].bitcast(jnp.bfloat16), sem_qkv.at[i])

    def o_copies():
        return [pltpu.make_async_copy(wo_hbm.at[:, pl.ds(n * 128, 128)],
                                      wo.at[n].bitcast(jnp.bfloat16), sem_o.at[0]) for n in range(ND)]

    for f in range(NCH):
        for c in glu_copies(f):
            c.start()
    for i, hbm in enumerate((wq_hbm, wk_hbm, wv_hbm)):
        qkv_copy(i, hbm).start()
    for c in o_copies():
        c.start()

    def ln_body(i, carry):
        r = pl.multiple_of(i * 128, 128)
        x = x_ref[pl.ds(r, 128), :].astype(jnp.float32)
        m = jnp.mean(x, axis=-1, keepdims=True)
        xc = x - m
        v = jnp.mean(xc * xc, axis=-1, keepdims=True)
        xn_scr[pl.ds(r, 128), :] = xc / jnp.sqrt(v + 1e-05)
        return carry
    jax.lax.fori_loop(0, S // 128, ln_body, 0)

    for f in range(NCH):
        for c in glu_copies(f):
            c.wait()
        xb = _bf16(xn_scr[0:_PRE, :])
        hs = []
        for j in range(TPC):
            c = f * TPC + j
            g = _dot(xb, _w(wg[c]))
            u = _dot(xb, _w(wu[c]))
            hs.append(_bf16(_sigmoid(g) * u))
        h = jnp.concatenate(hs, axis=1)
        for n in range(ND):
            y = _dot(h, _w(wd[n, f * (_FCH // 2):(f + 1) * (_FCH // 2), :]))
            if f == 0:
                acc_scr[:, n * 128:(n + 1) * 128] = y
            elif f < NCH - 1:
                acc_scr[:, n * 128:(n + 1) * 128] += y
            else:
                y = acc_scr[:, n * 128:(n + 1) * 128] + y
                g_scr[0:_PRE, n * 128:(n + 1) * 128] = y * _sigmoid(y)

    for i, hbm in enumerate((wq_hbm, wk_hbm, wv_hbm)):
        qkv_copy(i, hbm).wait()

        def conv(gi, carry, i=i):
            base = pl.multiple_of(gi * (8 * H), 8 * H)
            r = pl.multiple_of(gi * 8, 8)
            for j in range(H // 2):
                a = stg[i, pl.ds(base + j, 8, stride=H), :]
                b = stg[i, pl.ds(base + H // 2 + j, 8, stride=H), :]
                wqkv[i * H + 2 * j, pl.ds(r, 8), :] = (a & jnp.uint32(0xFFFF)) | (b << 16)
                wqkv[i * H + 2 * j + 1, pl.ds(r, 8), :] = (a >> 16) | (b & jnp.uint32(0xFFFF0000))
            return carry
        jax.lax.fori_loop(0, D // 16, conv, 0)
    for c in o_copies():
        c.wait()

    L = M + SEG
    LP = L + 8
    row = jax.lax.broadcasted_iota(jnp.int32, (LP, LP), 0)
    col = jax.lax.broadcasted_iota(jnp.int32, (LP, LP), 1)
    mask = ((row < M) | (row >= col)) & (col < L)

    def attn(q, k, v):
        s = jax.lax.dot_general(_bf16(q), _bf16(k), (((1,), (1,)), ((), ())),
                                preferred_element_type=jnp.float32) * scale
        s = jnp.where(mask, s, -1000000000.0)
        m = jnp.max(s, axis=-1, keepdims=True)
        e = jnp.exp(s - m)
        p = e / jnp.sum(e, axis=-1, keepdims=True)
        return _dot(_bf16(p), _bf16(v))

    GT = (S - _PRE) // (S // (2 * SEG))

    def pair(t, mem):
        r0 = pl.multiple_of(t * (2 * SEG), 2 * SEG)
        rg = pl.multiple_of(_PRE + t * GT, 8)
        xg = _bf16(xn_scr[pl.ds(rg, GT), :])
        hs = []
        for c in range(NF):
            g = _dot(xg, _w(wg[c]))
            u = _dot(xg, _w(wu[c]))
            hs.append(_bf16(_sigmoid(g) * u))
        h = jnp.concatenate(hs, axis=1)
        for n in range(ND):
            y = _dot(h, _w(wd[n]))
            g_scr[pl.ds(rg, GT), n * 128:(n + 1) * 128] = y * _sigmoid(y)

        lhs = _bf16(jnp.concatenate([mem, xn_scr[pl.ds(r0, 40), :]], axis=0))
        for hh in range(H):
            q = _dot(lhs, _w(wqkv[hh]))
            k = _dot(lhs, _w(wqkv[H + hh]))
            v = _dot(lhs, _w(wqkv[2 * H + hh]))
            cq[hh] = q[L:LP]
            ck[hh] = k[L:LP]
            cv[hh] = v[L:LP]
            o = attn(q, k, v)
            oa[:, hh * 128:(hh + 1) * 128] = _bf16(o[0:32])
            co[hh] = o[32:40]
        ya = jnp.concatenate([_dot(oa[...], _w(wo[n])) for n in range(ND)], axis=1)
        mem = ya[0:M]
        lhs = _bf16(jnp.concatenate([mem, xn_scr[pl.ds(r0 + 40, 24), :]], axis=0))
        for hh in range(H):
            q = _dot(lhs, _w(wqkv[hh]))
            k = _dot(lhs, _w(wqkv[H + hh]))
            v = _dot(lhs, _w(wqkv[2 * H + hh]))
            cqh, ckh, cvh = cq[hh], ck[hh], cv[hh]
            q = jnp.concatenate([q[0:8], cqh, q[8:32], cqh], axis=0)
            k = jnp.concatenate([k[0:8], ckh, k[8:32], ckh], axis=0)
            v = jnp.concatenate([v[0:8], cvh, v[8:32], cvh], axis=0)
            o = attn(q, k, v)
            ob[:, hh * 128:(hh + 1) * 128] = _bf16(jnp.concatenate([o[0:8], co[hh], o[8:40]], axis=0))
        yb = jnp.concatenate([_dot(ob[...], _w(wo[n])) for n in range(ND)], axis=1)
        mem = yb[0:M]
        s = jnp.concatenate([ya[8:32], yb[8:48]], axis=0)
        x = x_ref[pl.ds(r0, 2 * SEG), :].astype(jnp.float32)
        out_ref[pl.ds(r0, 2 * SEG), :] = (x + s * g_scr[pl.ds(r0, 2 * SEG), :]).astype(out_ref.dtype)
        return mem

    jax.lax.fori_loop(0, S // (2 * SEG), pair, mem0_ref[...].astype(jnp.float32))


@functools.partial(jax.jit, static_argnames=("A_seg_len",))
def pallas_recurrent_scan__memory_aug_recurrent_mem_tr__glu_gated_glu__prompt_kernel(
    A_x, A_mem0, A_Wq, A_Wk, A_Wv, A_Wo, A_seg_len, B_x, B_w_gate, B_w_up, B_w_down,
):
    del B_x
    B, S, D = A_x.shape
    H, Dh = A_Wq.shape[1], A_Wq.shape[2]
    M = A_mem0.shape[1]
    SEG = A_seg_len
    F = B_w_gate.shape[1]
    assert B == 1 and Dh == 128 and M == 8 and SEG == 32
    x = A_x.reshape(S, D)
    mem0 = A_mem0.reshape(M, D)
    wq = A_Wq.reshape(D * H, Dh)
    wk = A_Wk.reshape(D * H, Dh)
    wv = A_Wv.reshape(D * H, Dh)
    wo = A_Wo.reshape(H * Dh, D)
    u32, f32, bf16 = jnp.uint32, jnp.float32, jnp.bfloat16
    anyspec = pl.BlockSpec(memory_space=pl.ANY)
    out = pl.pallas_call(
        functools.partial(_kernel, S=S, D=D, H=H, M=M, SEG=SEG, F=F),
        out_shape=jax.ShapeDtypeStruct((S, D), A_x.dtype),
        in_specs=[pl.BlockSpec(memory_space=pltpu.VMEM), pl.BlockSpec(memory_space=pltpu.VMEM)] + [anyspec] * 7,
        out_specs=pl.BlockSpec(memory_space=pltpu.VMEM),
        scratch_shapes=[
            pltpu.VMEM((3 * H, D // 2, 128), u32),
            pltpu.VMEM((D // 128, H * Dh // 2, 128), u32),
            pltpu.VMEM((F // 128, D // 2, 128), u32),
            pltpu.VMEM((F // 128, D // 2, 128), u32),
            pltpu.VMEM((D // 128, F // 2, 128), u32),
            pltpu.VMEM((3, D * H // 2, 128), u32),
            pltpu.VMEM((S, D), f32),
            pltpu.VMEM((S, D), f32),
            pltpu.VMEM((_PRE, D), f32),
            pltpu.VMEM((H, 8, 128), f32),
            pltpu.VMEM((H, 8, 128), f32),
            pltpu.VMEM((H, 8, 128), f32),
            pltpu.VMEM((H, 8, 128), f32),
            pltpu.VMEM((32, H * Dh), bf16),
            pltpu.VMEM((48, H * Dh), bf16),
            pltpu.SemaphoreType.DMA((F // _FCH,)),
            pltpu.SemaphoreType.DMA((3,)),
            pltpu.SemaphoreType.DMA((1,)),
        ],
        compiler_params=pltpu.CompilerParams(vmem_limit_bytes=120 * 1024 * 1024),
    )(x, mem0, wq, wk, wv, wo, B_w_gate, B_w_up, B_w_down)
    return out.reshape(B, S, D)
```

```python
import functools

import jax
import jax.numpy as jnp
import jax.experimental.pallas as pl
import jax.experimental.pallas.tpu as pltpu

_PRE = 1024
_FCH = 512
_GRP = 8
_XCH = 512


def _sigmoid(x):
    return 1.0 / (1.0 + jnp.exp(-x))


def _bf16(x):
    return x.astype(jnp.bfloat16)


def _w(ref_val):
    return pltpu.bitcast(ref_val, jnp.bfloat16)


def _dot(a, b):
    return jnp.dot(a, b, preferred_element_type=jnp.float32)


def _kernel(mem0_ref, x_hbm, wq_hbm, wk_hbm, wv_hbm, wo_hbm, wg_hbm, wu_hbm, wd_hbm,
            out_hbm,
            wqkv, wo, wg, wu, wd, stg, x_scr, xn_scr, g_scr, acc_scr, out_scr,
            cq, ck, cv, co, oa, ob, q_s, k_s, v_s, lhs_s, xg_s, h_s,
            sem_x, sem_glu, sem_qkv, sem_o, sem_out,
            *, S, D, H, M, SEG, F):
    NF = F // 128
    ND = D // 128
    NCH = F // _FCH
    TPC = _FCH // 128
    NXC = S // _XCH
    scale = 128 ** (-0.5)

    def x_copy(i):
        return pltpu.make_async_copy(x_hbm.at[pl.ds(i * _XCH, _XCH), :], x_scr.at[pl.ds(i * _XCH, _XCH), :],
                                     sem_x.at[i])

    def glu_copies(f):
        cps = []
        for j in range(TPC):
            c = f * TPC + j
            cps.append(pltpu.make_async_copy(
                wg_hbm.at[:, pl.ds(c * 128, 128)], wg.at[c].bitcast(jnp.bfloat16), sem_glu.at[f]))
            cps.append(pltpu.make_async_copy(
                wu_hbm.at[:, pl.ds(c * 128, 128)], wu.at[c].bitcast(jnp.bfloat16), sem_glu.at[f]))
        for n in range(ND):
            cps.append(pltpu.make_async_copy(
                wd_hbm.at[pl.ds(f * _FCH, _FCH), pl.ds(n * 128, 128)],
                wd.at[n, pl.ds(f * (_FCH // 2), _FCH // 2), :].bitcast(jnp.bfloat16), sem_glu.at[f]))
        return cps

    def qkv_copies(i):
        w32 = (wq_hbm, wk_hbm, wv_hbm)[i].bitcast(jnp.uint32)
        return [pltpu.make_async_copy(w32.at[:, j, :], stg.at[i, j], sem_qkv.at[i]) for j in range(H // 2)]

    def o_copies():
        return [pltpu.make_async_copy(wo_hbm.at[:, pl.ds(n * 128, 128)],
                                      wo.at[n].bitcast(jnp.bfloat16), sem_o.at[0]) for n in range(ND)]

    def out_copy(r0, rows):
        return pltpu.make_async_copy(out_scr.at[pl.ds(r0, rows), :], out_hbm.at[pl.ds(r0, rows), :], sem_out.at[0])

    def layernorm(i):
        for r in range(i * _XCH, (i + 1) * _XCH, 128):
            x = x_scr[r:r + 128, :].astype(jnp.float32)
            m = jnp.mean(x, axis=-1, keepdims=True)
            xc = x - m
            v = jnp.mean(xc * xc, axis=-1, keepdims=True)
            xn_scr[r:r + 128, :] = xc / jnp.sqrt(v + 1e-05)

    def convert(i):
        for gi in range(D // 16):
            for j in range(H // 2):
                a = stg[i, j, pl.ds(gi * 16, 8, stride=2), :]
                b = stg[i, j, pl.ds(gi * 16 + 1, 8, stride=2), :]
                wqkv[i * H + 2 * j, gi * 8:gi * 8 + 8, :] = (a & jnp.uint32(0xFFFF)) | (b << 16)
                wqkv[i * H + 2 * j + 1, gi * 8:gi * 8 + 8, :] = (a >> 16) | (b & jnp.uint32(0xFFFF0000))

    NPX = _PRE // _XCH
    for i in range(NPX):
        x_copy(i).start()
    for f in range(2):
        for c in glu_copies(f):
            c.start()
    for i in range(NPX):
        x_copy(i).wait()
        layernorm(i)

    late = [("x", i) for i in range(NPX, NXC)]
    for f in range(NCH):
        for c in glu_copies(f):
            c.wait()
        if f + 2 < NCH:
            for c in glu_copies(f + 2):
                c.start()
        if f < 3:
            for c in qkv_copies(f):
                c.start()
        if f == 3:
            for c in o_copies():
                c.start()
            for i in range(NPX, NXC):
                x_copy(i).start()
        if f >= NCH - 3:
            i = f - (NCH - 3)
            for c in qkv_copies(i):
                c.wait()
        if f == NCH - 1:
            for i in range(NPX, NXC):
                x_copy(i).wait()
        xb = _bf16(xn_scr[0:_PRE, :])
        hs = []
        for j in range(TPC):
            c = f * TPC + j
            g = _dot(xb, _w(wg[c]))
            u = _dot(xb, _w(wu[c]))
            hs.append(_bf16(_sigmoid(g) * u))
        h = jnp.concatenate(hs, axis=1)
        if f >= NCH - 3:
            convert(f - (NCH - 3))
        if f == NCH - 1:
            for i in range(NPX, NXC):
                layernorm(i)
        for n in range(ND):
            y = _dot(h, _w(wd[n, f * (_FCH // 2):(f + 1) * (_FCH // 2), :]))
            if f == 0:
                acc_scr[:, n * 128:(n + 1) * 128] = y
            elif f < NCH - 1:
                acc_scr[:, n * 128:(n + 1) * 128] += y
            else:
                y = acc_scr[:, n * 128:(n + 1) * 128] + y
                g_scr[0:_PRE, n * 128:(n + 1) * 128] = y * _sigmoid(y)
    for c in o_copies():
        c.wait()

    L = M + SEG
    LP = L + 8
    row = jax.lax.broadcasted_iota(jnp.int32, (LP, LP), 0)
    col = jax.lax.broadcasted_iota(jnp.int32, (LP, LP), 1)
    mask = ((row < M) | (row >= col)) & (col < L)
    G = _GRP
    NG = H // G
    maskg = jnp.concatenate([mask] * G, axis=0)

    def attn_group(g0, fillers):
        ss = []
        for hh in range(g0, g0 + G):
            cs = slice(hh * 128, (hh + 1) * 128)
            ss.append(jax.lax.dot_general(q_s[:, cs], k_s[:, cs], (((1,), (1,)), ((), ())),
                                          preferred_element_type=jnp.float32))
        fillers()
        s = jnp.concatenate(ss, axis=0) * scale
        s = jnp.where(maskg, s, -1000000000.0)
        m = jnp.max(s, axis=-1, keepdims=True)
        e = jnp.exp(s - m)
        p = _bf16(e / jnp.sum(e, axis=-1, keepdims=True))
        fillers()
        return [_dot(p[i * LP:(i + 1) * LP], v_s[:, (g0 + i) * 128:(g0 + i + 1) * 128]) for i in range(G)]

    NIT = S // (2 * SEG)
    GT = (S - _PRE) // NIT

    def pair(t, mem):
        r0 = pl.multiple_of(t * (2 * SEG), 2 * SEG)
        rg = pl.multiple_of(_PRE + t * GT, 8)
        xg_s[...] = _bf16(xn_scr[pl.ds(rg, GT), :])

        def glu_up(c):
            g = _dot(xg_s[...], _w(wg[c]))
            u = _dot(xg_s[...], _w(wu[c]))
            h_s[:, c * 128:(c + 1) * 128] = _bf16(_sigmoid(g) * u)

        def glu_down(n):
            y = _dot(h_s[...], _w(wd[n]))
            g_scr[pl.ds(rg, GT), n * 128:(n + 1) * 128] = y * _sigmoid(y)

        def make_fillers(tasks, nslots):
            state = {"slot": 0, "done": 0}
            def f():
                state["slot"] += 1
                upto = (len(tasks) * state["slot"]) // nslots
                while state["done"] < upto:
                    tasks[state["done"]]()
                    state["done"] += 1
            return f

        lhs_s[...] = _bf16(jnp.concatenate([mem, xn_scr[pl.ds(r0, 40), :]], axis=0))
        for hh in range(H):
            cs = slice(hh * 128, (hh + 1) * 128)
            for i, (dst, c_) in enumerate(((q_s, cq), (k_s, ck), (v_s, cv))):
                y = _dot(lhs_s[...], _w(wqkv[i * H + hh]))
                dst[:, cs] = _bf16(y)
                c_[hh] = y[L:LP]
        fill = make_fillers([functools.partial(glu_up, c) for c in range(NF)], 2 * NG)
        for gi in range(NG):
            os_ = attn_group(gi * G, fill)
            for i, o in enumerate(os_):
                hh = gi * G + i
                oa[:, hh * 128:(hh + 1) * 128] = _bf16(o[0:32])
                co[hh] = o[32:40]
        ya = jnp.concatenate([_dot(oa[...], _w(wo[n])) for n in range(ND)], axis=1)
        mem = ya[0:M]
        lhs_s[0:32, :] = _bf16(jnp.concatenate([mem, xn_scr[pl.ds(r0 + 40, 24), :]], axis=0))
        for hh in range(H):
            cs = slice(hh * 128, (hh + 1) * 128)
            for i, (dst, c_) in enumerate(((q_s, cq), (k_s, ck), (v_s, cv))):
                y = _dot(lhs_s[0:32, :], _w(wqkv[i * H + hh]))
                cy = c_[hh]
                dst[:, cs] = _bf16(jnp.concatenate([y[0:8], cy, y[8:32], cy], axis=0))
        fill = make_fillers([functools.partial(glu_down, n) for n in range(ND)], 2 * NG)
        for gi in range(NG):
            os_ = attn_group(gi * G, fill)
            for i, o in enumerate(os_):
                hh = gi * G + i
                ob[:, hh * 128:(hh + 1) * 128] = _bf16(jnp.concatenate([o[0:8], co[hh], o[8:40]], axis=0))
        yb = jnp.concatenate([_dot(ob[...], _w(wo[n])) for n in range(ND)], axis=1)
        mem = yb[0:M]
        s = jnp.concatenate([ya[8:32], yb[8:48]], axis=0)
        x = x_scr[pl.ds(r0, 2 * SEG), :].astype(jnp.float32)
        out_scr[pl.ds(r0, 2 * SEG), :] = (x + s * g_scr[pl.ds(r0, 2 * SEG), :]).astype(out_scr.dtype)
        out_copy(r0, 2 * SEG).start()
        return mem

    NRUN = NIT
    jax.lax.fori_loop(0, NRUN, pair, mem0_ref[...].astype(jnp.float32))
    for t in range(NRUN):
        out_copy(t * 2 * SEG, 2 * SEG).wait()


@functools.partial(jax.jit, static_argnames=("A_seg_len",))
def pallas_recurrent_scan__memory_aug_recurrent_mem_tr__glu_gated_glu__prompt_kernel(
    A_x, A_mem0, A_Wq, A_Wk, A_Wv, A_Wo, A_seg_len, B_x, B_w_gate, B_w_up, B_w_down,
):
    del B_x
    B, S, D = A_x.shape
    H, Dh = A_Wq.shape[1], A_Wq.shape[2]
    M = A_mem0.shape[1]
    SEG = A_seg_len
    F = B_w_gate.shape[1]
    assert B == 1 and Dh == 128 and M == 8 and SEG == 32
    x = A_x.reshape(S, D)
    mem0 = A_mem0.reshape(M, D)
    wo = A_Wo.reshape(H * Dh, D)
    u32, f32, bf16 = jnp.uint32, jnp.float32, jnp.bfloat16
    anyspec = pl.BlockSpec(memory_space=pl.ANY)
    out = pl.pallas_call(
        functools.partial(_kernel, S=S, D=D, H=H, M=M, SEG=SEG, F=F),
        out_shape=jax.ShapeDtypeStruct((S, D), A_x.dtype),
        in_specs=[pl.BlockSpec(memory_space=pltpu.VMEM)] + [anyspec] * 8,
        out_specs=anyspec,
        scratch_shapes=[
            pltpu.VMEM((3 * H, D // 2, 128), u32),
            pltpu.VMEM((D // 128, H * Dh // 2, 128), u32),
            pltpu.VMEM((F // 128, D // 2, 128), u32),
            pltpu.VMEM((F // 128, D // 2, 128), u32),
            pltpu.VMEM((D // 128, F // 2, 128), u32),
            pltpu.VMEM((3, H // 2, D, 128), u32),
            pltpu.VMEM((S, D), bf16),
            pltpu.VMEM((S, D), f32),
            pltpu.VMEM((S, D), f32),
            pltpu.VMEM((_PRE, D), f32),
            pltpu.VMEM((S, D), bf16),
            pltpu.VMEM((H, 8, 128), f32),
            pltpu.VMEM((H, 8, 128), f32),
            pltpu.VMEM((H, 8, 128), f32),
            pltpu.VMEM((H, 8, 128), f32),
            pltpu.VMEM((32, H * Dh), bf16),
            pltpu.VMEM((48, H * Dh), bf16),
            pltpu.VMEM((48, H * Dh), bf16),
            pltpu.VMEM((48, H * Dh), bf16),
            pltpu.VMEM((48, H * Dh), bf16),
            pltpu.VMEM((48, D), bf16),
            pltpu.VMEM(((S - _PRE) // (S // (2 * SEG)), D), bf16),
            pltpu.VMEM(((S - _PRE) // (S // (2 * SEG)), F), bf16),
            pltpu.SemaphoreType.DMA((S // _XCH,)),
            pltpu.SemaphoreType.DMA((F // _FCH,)),
            pltpu.SemaphoreType.DMA((3,)),
            pltpu.SemaphoreType.DMA((1,)),
            pltpu.SemaphoreType.DMA((1,)),
        ],
        compiler_params=pltpu.CompilerParams(vmem_limit_bytes=124 * 1024 * 1024),
    )(mem0, x, A_Wq, A_Wk, A_Wv, wo, B_w_gate, B_w_up, B_w_down)
    return out.reshape(B, S, D)
```

```python
import functools

import jax
import jax.numpy as jnp
import jax.experimental.pallas as pl
import jax.experimental.pallas.tpu as pltpu

_PRE = 1024
_FCH = 512
_GRP = 8
_SLOTS = [4,2,2,2,2,2,2,2,2,2,2, 2,2,1,1,1,1,1,1,1,1,0]
_XCH = 256


def _sigmoid(x):
    return 1.0 / (1.0 + jnp.exp(-x))


def _bf16(x):
    return x.astype(jnp.bfloat16)


def _w(ref_val):
    return pltpu.bitcast(ref_val, jnp.bfloat16)


def _p(val):
    return pltpu.bitcast(val, jnp.uint32)


def _dot(a, b):
    return jnp.dot(a, b, preferred_element_type=jnp.float32)


def _kernel(mem0_ref, x_hbm, wq_hbm, wk_hbm, wv_hbm, wo_hbm, wg_hbm, wu_hbm, wd_hbm,
            out_hbm,
            wqkv, wo, wg, wu, wd, stg, x_scr, xn_scr, g_scr, acc_scr, out_scr,
            cq, ck, cv, co, oa, ob, q_s, k_s, v_s, lhs_s, xg_s, h_s, xb_s, hp_s,
            sem_x, sem_u0, sem_glu, sem_qkv, sem_o, sem_out,
            *, S, D, H, M, SEG, F):
    NF = F // 128
    ND = D // 128
    NCH = F // _FCH
    TPC = _FCH // 128
    NXC = S // _XCH
    scale = 128 ** (-0.5)

    def x_copy(i):
        return pltpu.make_async_copy(x_hbm.at[pl.ds(i * _XCH, _XCH), :], x_scr.at[pl.ds(i * _XCH, _XCH), :],
                                     sem_x.at[i])

    def up_copies(f):
        cps = []
        for j in range(TPC):
            c = f * TPC + j
            cps.append(pltpu.make_async_copy(
                wg_hbm.at[:, pl.ds(c * 128, 128)], wg.at[c].bitcast(jnp.bfloat16), sem_glu.at[f]))
            cps.append(pltpu.make_async_copy(
                wu_hbm.at[:, pl.ds(c * 128, 128)], wu.at[c].bitcast(jnp.bfloat16), sem_glu.at[f]))
        return cps

    def down_copies(f):
        return [pltpu.make_async_copy(
            wd_hbm.at[pl.ds(f * _FCH, _FCH), pl.ds(n * 128, 128)],
            wd.at[n, pl.ds(f * (_FCH // 2), _FCH // 2), :].bitcast(jnp.bfloat16), sem_glu.at[NCH + f])
            for n in range(ND)]

    def qkv_copies(i):
        w32 = (wq_hbm, wk_hbm, wv_hbm)[i].bitcast(jnp.uint32)
        return [pltpu.make_async_copy(w32.at[:, j, :], stg.at[i, j], sem_qkv.at[i]) for j in range(H // 2)]

    def o_copies():
        return [pltpu.make_async_copy(wo_hbm.at[:, pl.ds(n * 128, 128)],
                                      wo.at[n].bitcast(jnp.bfloat16), sem_o.at[0]) for n in range(ND)]

    def out_copy(r0, rows):
        return pltpu.make_async_copy(out_scr.at[pl.ds(r0, rows), :], out_hbm.at[pl.ds(r0, rows), :], sem_out.at[0])

    def layernorm(i):
        for r in range(i * _XCH, (i + 1) * _XCH, 128):
            x = x_scr[r:r + 128, :].astype(jnp.float32)
            m = jnp.mean(x, axis=-1, keepdims=True)
            xc = x - m
            v = jnp.mean(xc * xc, axis=-1, keepdims=True)
            xn_scr[r:r + 128, :] = xc / jnp.sqrt(v + 1e-05)

    def convert(i):
        for gi in range(D // 16):
            for j in range(H // 2):
                a = stg[i, j, pl.ds(gi * 16, 8, stride=2), :]
                b = stg[i, j, pl.ds(gi * 16 + 1, 8, stride=2), :]
                wqkv[i * H + 2 * j, gi * 8:gi * 8 + 8, :] = (a & jnp.uint32(0xFFFF)) | (b << 16)
                wqkv[i * H + 2 * j + 1, gi * 8:gi * 8 + 8, :] = (a >> 16) | (b & jnp.uint32(0xFFFF0000))

    NPX = _PRE // _XCH

    def up0(j):
        return [pltpu.make_async_copy(wg_hbm.at[:, pl.ds(j * 128, 128)], wg.at[j].bitcast(jnp.bfloat16), sem_u0.at[j]),
                pltpu.make_async_copy(wu_hbm.at[:, pl.ds(j * 128, 128)], wu.at[j].bitcast(jnp.bfloat16), sem_u0.at[j])]

    def up_tile(c, j, m0, mb):
        xb = _w(xb_s[m0 // 2:(m0 + mb) // 2, :])
        g = _dot(xb, _w(wg[c]))
        u = _dot(xb, _w(wu[c]))
        hp_s[m0 // 2:(m0 + mb) // 2, j * 128:(j + 1) * 128] = _p(_bf16(_sigmoid(g) * u))

    x_copy(0).start()
    for c in up0(0):
        c.start()
    for i in range(1, NPX):
        x_copy(i).start()
    for i in range(NPX):
        x_copy(i).wait()
        if i + 1 < TPC:
            for c in up0(i + 1):
                c.start()
        if i == NPX - 1:
            for c in down_copies(0):
                c.start()
        layernorm(i)
        xb_s[i * (_XCH // 2):(i + 1) * (_XCH // 2), :] = _p(_bf16(xn_scr[i * _XCH:(i + 1) * _XCH, :]))
        if i == 0:
            for c in up0(0):
                c.wait()
        up_tile(0, 0, i * _XCH, _XCH)

    for f in range(NCH):
        if f == 0:
            for j in range(1, TPC):
                for c in up0(j):
                    c.wait()
                if j == 1:
                    for c in up_copies(1) + down_copies(1):
                        c.start()
                up_tile(j, j, 0, _PRE)
        else:
            for c in up_copies(f):
                c.wait()
        if f + 2 < NCH:
            for c in up_copies(f + 2) + down_copies(f + 2):
                c.start()
        if f < 3:
            for c in qkv_copies(f):
                c.start()
        if f == 3:
            for c in o_copies():
                c.start()
            for i in range(NPX, NXC):
                x_copy(i).start()
        if f >= NCH - 3:
            i = f - (NCH - 3)
            for c in qkv_copies(i):
                c.wait()
        if f == NCH - 1:
            for i in range(NPX, NXC):
                x_copy(i).wait()
        MB = 256
        if f > 0:
            for j in range(TPC):
                up_tile(f * TPC + j, j, 0, _PRE)
        if f >= NCH - 3:
            convert(f - (NCH - 3))
        if f == NCH - 1:
            for i in range(NPX, NXC):
                layernorm(i)
        for c in down_copies(f):
            c.wait()
        for m0 in range(0, _PRE, MB):
          ms = slice(m0, m0 + MB)
          for n in range(ND):
            y = _dot(_w(hp_s[m0 // 2:(m0 + MB) // 2, :]), _w(wd[n, f * (_FCH // 2):(f + 1) * (_FCH // 2), :]))
            if f == 0:
                acc_scr[ms, n * 128:(n + 1) * 128] = y
            elif f < NCH - 1:
                acc_scr[ms, n * 128:(n + 1) * 128] += y
            else:
                y = acc_scr[ms, n * 128:(n + 1) * 128] + y
                g_scr[ms, n * 128:(n + 1) * 128] = y * _sigmoid(y)
    for c in o_copies():
        c.wait()

    L = M + SEG
    LP = L + 8
    row = jax.lax.broadcasted_iota(jnp.int32, (LP, LP), 0)
    col = jax.lax.broadcasted_iota(jnp.int32, (LP, LP), 1)
    mask = ((row < M) | (row >= col)) & (col < L)
    G = _GRP
    NG = H // G
    maskg = jnp.concatenate([mask] * G, axis=0)

    def attn_group(g0, fillers):
        ss = []
        for hh in range(g0, g0 + G):
            cs = slice(hh * 128, (hh + 1) * 128)
            ss.append(jax.lax.dot_general(_w(q_s[:, cs]), _w(k_s[:, cs]), (((1,), (1,)), ((), ())),
                                          preferred_element_type=jnp.float32))
        fillers()
        s = jnp.concatenate(ss, axis=0) * scale
        s = jnp.where(maskg, s, -1000000000.0)
        m = jnp.max(s, axis=-1, keepdims=True)
        e = jnp.exp(s - m)
        p = _bf16(e / jnp.sum(e, axis=-1, keepdims=True))
        fillers()
        return [_dot(p[i * LP:(i + 1) * LP], _w(v_s[:, (g0 + i) * 128:(g0 + i + 1) * 128])) for i in range(G)]

    NIT = S // (2 * SEG)
    GT = (S - _PRE) // NIT

    def pair(t, mem):
        r0 = pl.multiple_of(t * (2 * SEG), 2 * SEG)
        rg = pl.multiple_of(_PRE + t * GT, 8)
        xg_s[...] = _p(_bf16(xn_scr[pl.ds(rg, GT), :]))

        def glu_up(c):
            g = _dot(_w(xg_s[...]), _w(wg[c]))
            u = _dot(_w(xg_s[...]), _w(wu[c]))
            h_s[:, c * 128:(c + 1) * 128] = _p(_bf16(_sigmoid(g) * u))

        def glu_down(n):
            y = _dot(_w(h_s[...]), _w(wd[n]))
            g_scr[pl.ds(rg, GT), n * 128:(n + 1) * 128] = y * _sigmoid(y)

        tasks = [functools.partial(glu_up, c) for c in range(NF)] + [functools.partial(glu_down, n) for n in range(ND)]
        counts = list(_SLOTS)
        assert sum(counts) == len(tasks), (sum(counts), len(tasks))
        state = {"slot": 0, "done": 0}

        def fill():
            for _ in range(counts[state["slot"]]):
                tasks[state["done"]]()
                state["done"] += 1
            state["slot"] += 1

        lhs_s[...] = _p(_bf16(jnp.concatenate([mem, xn_scr[pl.ds(r0, 40), :]], axis=0)))
        fill()
        for hh in range(H):
            cs = slice(hh * 128, (hh + 1) * 128)
            for i, (dst, c_) in enumerate(((q_s, cq), (k_s, ck), (v_s, cv))):
                y = _dot(_w(lhs_s[...]), _w(wqkv[i * H + hh]))
                dst[:, cs] = _p(_bf16(y))
                c_[hh] = y[L:LP]
        fill()
        for gi in range(NG):
            os_ = attn_group(gi * G, fill)
            for i, o in enumerate(os_):
                hh = gi * G + i
                oa[:, hh * 128:(hh + 1) * 128] = _p(_bf16(o[0:32]))
                co[hh] = o[32:40]
        fill()
        ya = jnp.concatenate([_dot(_w(oa[...]), _w(wo[n])) for n in range(ND)], axis=1)
        mem = ya[0:M]
        lhs_s[0:16, :] = _p(_bf16(jnp.concatenate([mem, xn_scr[pl.ds(r0 + 40, 24), :]], axis=0)))
        fill()
        for hh in range(H):
            cs = slice(hh * 128, (hh + 1) * 128)
            for i, (dst, c_) in enumerate(((q_s, cq), (k_s, ck), (v_s, cv))):
                y = _dot(_w(lhs_s[0:16, :]), _w(wqkv[i * H + hh]))
                cy = c_[hh]
                dst[:, cs] = _p(_bf16(jnp.concatenate([y[0:8], cy, y[8:32], cy], axis=0)))
        fill()
        for gi in range(NG):
            os_ = attn_group(gi * G, fill)
            for i, o in enumerate(os_):
                hh = gi * G + i
                ob[:, hh * 128:(hh + 1) * 128] = _p(_bf16(jnp.concatenate([o[0:8], co[hh], o[8:40]], axis=0)))
        fill()
        yb = jnp.concatenate([_dot(_w(ob[...]), _w(wo[n])) for n in range(ND)], axis=1)
        mem = yb[0:M]
        s = jnp.concatenate([ya[8:32], yb[8:48]], axis=0)
        x = x_scr[pl.ds(r0, 2 * SEG), :].astype(jnp.float32)
        out_scr[pl.ds(r0, 2 * SEG), :] = (x + s * g_scr[pl.ds(r0, 2 * SEG), :]).astype(out_scr.dtype)
        out_copy(r0, 2 * SEG).start()
        return mem

    NRUN = NIT
    jax.lax.fori_loop(0, NRUN, pair, mem0_ref[...].astype(jnp.float32))
    for t in range(NRUN):
        out_copy(t * 2 * SEG, 2 * SEG).wait()


@functools.partial(jax.jit, static_argnames=("A_seg_len",))
def pallas_recurrent_scan__memory_aug_recurrent_mem_tr__glu_gated_glu__prompt_kernel(
    A_x, A_mem0, A_Wq, A_Wk, A_Wv, A_Wo, A_seg_len, B_x, B_w_gate, B_w_up, B_w_down,
):
    del B_x
    B, S, D = A_x.shape
    H, Dh = A_Wq.shape[1], A_Wq.shape[2]
    M = A_mem0.shape[1]
    SEG = A_seg_len
    F = B_w_gate.shape[1]
    assert B == 1 and Dh == 128 and M == 8 and SEG == 32
    x = A_x.reshape(S, D)
    mem0 = A_mem0.reshape(M, D)
    wo = A_Wo.reshape(H * Dh, D)
    u32, f32, bf16 = jnp.uint32, jnp.float32, jnp.bfloat16
    anyspec = pl.BlockSpec(memory_space=pl.ANY)
    out = pl.pallas_call(
        functools.partial(_kernel, S=S, D=D, H=H, M=M, SEG=SEG, F=F),
        out_shape=jax.ShapeDtypeStruct((S, D), A_x.dtype),
        in_specs=[pl.BlockSpec(memory_space=pltpu.VMEM)] + [anyspec] * 8,
        out_specs=anyspec,
        scratch_shapes=[
            pltpu.VMEM((3 * H, D // 2, 128), u32),
            pltpu.VMEM((D // 128, H * Dh // 2, 128), u32),
            pltpu.VMEM((F // 128, D // 2, 128), u32),
            pltpu.VMEM((F // 128, D // 2, 128), u32),
            pltpu.VMEM((D // 128, F // 2, 128), u32),
            pltpu.VMEM((3, H // 2, D, 128), u32),
            pltpu.VMEM((S, D), bf16),
            pltpu.VMEM((S, D), f32),
            pltpu.VMEM((S, D), f32),
            pltpu.VMEM((_PRE, D), f32),
            pltpu.VMEM((S, D), bf16),
            pltpu.VMEM((H, 8, 128), f32),
            pltpu.VMEM((H, 8, 128), f32),
            pltpu.VMEM((H, 8, 128), f32),
            pltpu.VMEM((H, 8, 128), f32),
            pltpu.VMEM((16, H * Dh), u32),
            pltpu.VMEM((24, H * Dh), u32),
            pltpu.VMEM((24, H * Dh), u32),
            pltpu.VMEM((24, H * Dh), u32),
            pltpu.VMEM((24, H * Dh), u32),
            pltpu.VMEM((24, D), u32),
            pltpu.VMEM(((S - _PRE) // (S // (2 * SEG)) // 2, D), u32),
            pltpu.VMEM(((S - _PRE) // (S // (2 * SEG)) // 2, F), u32),
            pltpu.VMEM((_PRE // 2, D), u32),
            pltpu.VMEM((_PRE // 2, _FCH), u32),
            pltpu.SemaphoreType.DMA((S // _XCH,)),
            pltpu.SemaphoreType.DMA((_FCH // 128,)),
            pltpu.SemaphoreType.DMA((2 * (F // _FCH),)),
            pltpu.SemaphoreType.DMA((3,)),
            pltpu.SemaphoreType.DMA((1,)),
            pltpu.SemaphoreType.DMA((1,)),
        ],
        compiler_params=pltpu.CompilerParams(vmem_limit_bytes=124 * 1024 * 1024),
    )(mem0, x, A_Wq, A_Wk, A_Wv, wo, B_w_gate, B_w_up, B_w_down)
    return out.reshape(B, S, D)
```

```python
import functools

import jax
import jax.numpy as jnp
import jax.experimental.pallas as pl
import jax.experimental.pallas.tpu as pltpu

_PRE = 1024
_FCH = 512
_GRP = 8
_SLOTS = [4,2,2,2,2,2,2,2,2,2,2, 2,2,1,1,1,1,1,1,1,1,0]
_XCH = 256


def _sigmoid(x):
    return 1.0 / (1.0 + jnp.exp(-x))


def _bf16(x):
    return x.astype(jnp.bfloat16)


def _w(ref_val):
    return pltpu.bitcast(ref_val, jnp.bfloat16)


def _p(val):
    return pltpu.bitcast(val, jnp.uint32)


def _dot(a, b):
    return jnp.dot(a, b, preferred_element_type=jnp.float32)


def _kernel(mem0_ref, x_hbm, wq_hbm, wk_hbm, wv_hbm, wo_hbm, wg_hbm, wu_hbm, wd_hbm,
            out_hbm,
            wqkv, wo, wg, wu, wd, stg, x_scr, xn_scr, g_scr, acc_scr, out_scr,
            cq, ck, cv, co, oa, ob, q_s, k_s, v_s, lhs_s, xg_s, h_s, xb_s, hp_s,
            sem_x, sem_u0, sem_glu, sem_qkv, sem_o, sem_out,
            *, S, D, H, M, SEG, F):
    NF = F // 128
    ND = D // 128
    NCH = F // _FCH
    TPC = _FCH // 128
    NXC = S // _XCH
    scale = 128 ** (-0.5)

    def x_copy(i):
        return pltpu.make_async_copy(x_hbm.at[pl.ds(i * _XCH, _XCH), :], x_scr.at[pl.ds(i * _XCH, _XCH), :],
                                     sem_x.at[i])

    def up_copies(f):
        cps = []
        for j in range(TPC):
            c = f * TPC + j
            cps.append(pltpu.make_async_copy(
                wg_hbm.at[:, pl.ds(c * 128, 128)], wg.at[c].bitcast(jnp.bfloat16), sem_glu.at[f]))
            cps.append(pltpu.make_async_copy(
                wu_hbm.at[:, pl.ds(c * 128, 128)], wu.at[c].bitcast(jnp.bfloat16), sem_glu.at[f]))
        return cps

    def down_copies(f):
        return [pltpu.make_async_copy(
            wd_hbm.at[pl.ds(f * _FCH, _FCH), pl.ds(n * 128, 128)],
            wd.at[n, pl.ds(f * (_FCH // 2), _FCH // 2), :].bitcast(jnp.bfloat16), sem_glu.at[NCH + f])
            for n in range(ND)]

    def qkv_copies(i):
        w32 = (wq_hbm, wk_hbm, wv_hbm)[i].bitcast(jnp.uint32)
        return [pltpu.make_async_copy(w32.at[:, j, :], stg.at[i, j], sem_qkv.at[i]) for j in range(H // 2)]

    def o_copies():
        return [pltpu.make_async_copy(wo_hbm.at[:, pl.ds(n * 128, 128)],
                                      wo.at[n].bitcast(jnp.bfloat16), sem_o.at[0]) for n in range(ND)]

    def out_copy(r0, rows):
        return pltpu.make_async_copy(out_scr.at[pl.ds(r0, rows), :], out_hbm.at[pl.ds(r0, rows), :], sem_out.at[0])

    def layernorm(i):
        for r in range(i * _XCH, (i + 1) * _XCH, 128):
            x = x_scr[r:r + 128, :].astype(jnp.float32)
            m = jnp.mean(x, axis=-1, keepdims=True)
            xc = x - m
            v = jnp.mean(xc * xc, axis=-1, keepdims=True)
            xn_scr[r:r + 128, :] = xc / jnp.sqrt(v + 1e-05)

    def convert(i):
        for gi in range(D // 16):
            for j in range(H // 2):
                a = stg[i, j, pl.ds(gi * 16, 8, stride=2), :]
                b = stg[i, j, pl.ds(gi * 16 + 1, 8, stride=2), :]
                wqkv[i * H + 2 * j, gi * 8:gi * 8 + 8, :] = (a & jnp.uint32(0xFFFF)) | (b << 16)
                wqkv[i * H + 2 * j + 1, gi * 8:gi * 8 + 8, :] = (a >> 16) | (b & jnp.uint32(0xFFFF0000))

    NPX = _PRE // _XCH

    def up0(j):
        return [pltpu.make_async_copy(wg_hbm.at[:, pl.ds(j * 128, 128)], wg.at[j].bitcast(jnp.bfloat16), sem_u0.at[j]),
                pltpu.make_async_copy(wu_hbm.at[:, pl.ds(j * 128, 128)], wu.at[j].bitcast(jnp.bfloat16), sem_u0.at[j])]

    def up_tile(c, j, m0, mb):
        xb = _w(xb_s[m0 // 2:(m0 + mb) // 2, :])
        g = _dot(xb, _w(wg[c]))
        u = _dot(xb, _w(wu[c]))
        hp_s[m0 // 2:(m0 + mb) // 2, j * 128:(j + 1) * 128] = _p(_bf16(_sigmoid(g) * u))

    x_copy(0).start()
    for c in up0(0):
        c.start()
    for i in range(1, NPX):
        x_copy(i).start()
    for i in range(NPX):
        x_copy(i).wait()
        if i + 1 < TPC:
            for c in up0(i + 1):
                c.start()
        if i == NPX - 1:
            for c in down_copies(0):
                c.start()
        layernorm(i)
        xb_s[i * (_XCH // 2):(i + 1) * (_XCH // 2), :] = _p(_bf16(xn_scr[i * _XCH:(i + 1) * _XCH, :]))
        if i == 0:
            for c in up0(0):
                c.wait()
        up_tile(0, 0, i * _XCH, _XCH)

    for f in range(NCH):
        if f == 0:
            for j in range(1, TPC):
                for c in up0(j):
                    c.wait()
                if j == 1:
                    for c in up_copies(1) + down_copies(1):
                        c.start()
                up_tile(j, j, 0, _PRE)
        else:
            for c in up_copies(f):
                c.wait()
        if f + 2 < NCH:
            for c in up_copies(f + 2) + down_copies(f + 2):
                c.start()
        if f < 3:
            for c in qkv_copies(f):
                c.start()
        if f == 3:
            for c in o_copies():
                c.start()
            for i in range(NPX, NXC):
                x_copy(i).start()
        if f >= NCH - 3:
            i = f - (NCH - 3)
            for c in qkv_copies(i):
                c.wait()
        if f == NCH - 1:
            for i in range(NPX, NXC):
                x_copy(i).wait()
        MB = 256
        if f > 0:
            for j in range(TPC):
                up_tile(f * TPC + j, j, 0, _PRE)
        if f >= NCH - 3:
            convert(f - (NCH - 3))
        if f == NCH - 1:
            for i in range(NPX, NXC):
                layernorm(i)
        for c in down_copies(f):
            c.wait()
        for m0 in range(0, _PRE, MB):
          ms = slice(m0, m0 + MB)
          for n in range(ND):
            y = _dot(_w(hp_s[m0 // 2:(m0 + MB) // 2, :]), _w(wd[n, f * (_FCH // 2):(f + 1) * (_FCH // 2), :]))
            if f == 0:
                acc_scr[ms, n * 128:(n + 1) * 128] = y
            elif f < NCH - 1:
                acc_scr[ms, n * 128:(n + 1) * 128] += y
            else:
                y = acc_scr[ms, n * 128:(n + 1) * 128] + y
                g_scr[ms, n * 128:(n + 1) * 128] = y * _sigmoid(y)
    for c in o_copies():
        c.wait()

    L = M + SEG
    L2 = 2 * L
    row = jax.lax.broadcasted_iota(jnp.int32, (L2, L2), 0)
    col = jax.lax.broadcasted_iota(jnp.int32, (L2, L2), 1)
    rm = jnp.where(row >= L, row - L, row)
    cm = jnp.where(col >= L, col - L, col)
    mask = ((row >= L) == (col >= L)) & ((rm < M) | (rm >= cm))
    G = _GRP // 2
    NG = H // 2 // G
    maskg = jnp.concatenate([mask] * G, axis=0)

    def attn_group(p0, fillers):
        ss = []
        for pp in range(p0, p0 + G):
            ss.append(jax.lax.dot_general(_w(q_s[pp]), _w(k_s[pp]), (((1,), (1,)), ((), ())),
                                          preferred_element_type=jnp.float32))
        fillers()
        s = jnp.concatenate(ss, axis=0) * scale
        s = jnp.where(maskg, s, -1000000000.0)
        m = jnp.max(s, axis=-1, keepdims=True)
        e = jnp.exp(s - m)
        p = _bf16(e / jnp.sum(e, axis=-1, keepdims=True))
        fillers()
        outs = []
        for i in range(G):
            o = _dot(p[i * L2:(i + 1) * L2], _w(v_s[p0 + i]))
            outs += [o[0:L], o[L:L2]]
        return outs

    NIT = S // (2 * SEG)
    GT = (S - _PRE) // NIT

    def pair(t, mem):
        r0 = pl.multiple_of(t * (2 * SEG), 2 * SEG)
        rg = pl.multiple_of(_PRE + t * GT, 8)
        xg_s[...] = _p(_bf16(xn_scr[pl.ds(rg, GT), :]))

        def glu_up(c):
            g = _dot(_w(xg_s[...]), _w(wg[c]))
            u = _dot(_w(xg_s[...]), _w(wu[c]))
            h_s[:, c * 128:(c + 1) * 128] = _p(_bf16(_sigmoid(g) * u))

        def glu_down(n):
            y = _dot(_w(h_s[...]), _w(wd[n]))
            g_scr[pl.ds(rg, GT), n * 128:(n + 1) * 128] = y * _sigmoid(y)

        tasks = [functools.partial(glu_up, c) for c in range(NF)] + [functools.partial(glu_down, n) for n in range(ND)]
        counts = list(_SLOTS)
        assert sum(counts) == len(tasks), (sum(counts), len(tasks))
        state = {"slot": 0, "done": 0}

        def fill():
            for _ in range(counts[state["slot"]]):
                tasks[state["done"]]()
                state["done"] += 1
            state["slot"] += 1

        lhs_s[...] = _p(_bf16(jnp.concatenate([mem, xn_scr[pl.ds(r0, 40), :]], axis=0)))
        fill()
        for pp in range(H // 2):
            for i, (dst, c_) in enumerate(((q_s, cq), (k_s, ck), (v_s, cv))):
                ys = []
                for hh in (2 * pp, 2 * pp + 1):
                    y = _dot(_w(lhs_s[...]), _w(wqkv[i * H + hh]))
                    c_[hh] = y[L:L + 8]
                    ys.append(y[0:L])
                dst[pp] = _p(_bf16(jnp.concatenate(ys, axis=0)))
        fill()
        for gi in range(NG):
            os_ = attn_group(gi * G, fill)
            for i, o in enumerate(os_):
                hh = gi * G * 2 + i
                oa[:, hh * 128:(hh + 1) * 128] = _p(_bf16(o[0:32]))
                co[hh] = o[32:40]
        fill()
        ya = jnp.concatenate([_dot(_w(oa[...]), _w(wo[n])) for n in range(ND)], axis=1)
        mem = ya[0:M]
        lhs_s[0:16, :] = _p(_bf16(jnp.concatenate([mem, xn_scr[pl.ds(r0 + 40, 24), :]], axis=0)))
        fill()
        for pp in range(H // 2):
            for i, (dst, c_) in enumerate(((q_s, cq), (k_s, ck), (v_s, cv))):
                ys = []
                for hh in (2 * pp, 2 * pp + 1):
                    y = _dot(_w(lhs_s[0:16, :]), _w(wqkv[i * H + hh]))
                    ys += [y[0:8], c_[hh], y[8:32]]
                dst[pp] = _p(_bf16(jnp.concatenate(ys, axis=0)))
        fill()
        for gi in range(NG):
            os_ = attn_group(gi * G, fill)
            for i, o in enumerate(os_):
                hh = gi * G * 2 + i
                ob[:, hh * 128:(hh + 1) * 128] = _p(_bf16(jnp.concatenate([o[0:8], co[hh], o[8:40]], axis=0)))
        fill()
        yb = jnp.concatenate([_dot(_w(ob[...]), _w(wo[n])) for n in range(ND)], axis=1)
        mem = yb[0:M]
        s = jnp.concatenate([ya[8:32], yb[8:48]], axis=0)
        x = x_scr[pl.ds(r0, 2 * SEG), :].astype(jnp.float32)
        out_scr[pl.ds(r0, 2 * SEG), :] = (x + s * g_scr[pl.ds(r0, 2 * SEG), :]).astype(out_scr.dtype)
        out_copy(r0, 2 * SEG).start()
        return mem

    NRUN = NIT
    jax.lax.fori_loop(0, NRUN, pair, mem0_ref[...].astype(jnp.float32))
    for t in range(NRUN):
        out_copy(t * 2 * SEG, 2 * SEG).wait()


@functools.partial(jax.jit, static_argnames=("A_seg_len",))
def pallas_recurrent_scan__memory_aug_recurrent_mem_tr__glu_gated_glu__prompt_kernel(
    A_x, A_mem0, A_Wq, A_Wk, A_Wv, A_Wo, A_seg_len, B_x, B_w_gate, B_w_up, B_w_down,
):
    del B_x
    B, S, D = A_x.shape
    H, Dh = A_Wq.shape[1], A_Wq.shape[2]
    M = A_mem0.shape[1]
    SEG = A_seg_len
    F = B_w_gate.shape[1]
    assert B == 1 and Dh == 128 and M == 8 and SEG == 32
    x = A_x.reshape(S, D)
    mem0 = A_mem0.reshape(M, D)
    wo = A_Wo.reshape(H * Dh, D)
    u32, f32, bf16 = jnp.uint32, jnp.float32, jnp.bfloat16
    anyspec = pl.BlockSpec(memory_space=pl.ANY)
    out = pl.pallas_call(
        functools.partial(_kernel, S=S, D=D, H=H, M=M, SEG=SEG, F=F),
        out_shape=jax.ShapeDtypeStruct((S, D), A_x.dtype),
        in_specs=[pl.BlockSpec(memory_space=pltpu.VMEM)] + [anyspec] * 8,
        out_specs=anyspec,
        scratch_shapes=[
            pltpu.VMEM((3 * H, D // 2, 128), u32),
            pltpu.VMEM((D // 128, H * Dh // 2, 128), u32),
            pltpu.VMEM((F // 128, D // 2, 128), u32),
            pltpu.VMEM((F // 128, D // 2, 128), u32),
            pltpu.VMEM((D // 128, F // 2, 128), u32),
            pltpu.VMEM((3, H // 2, D, 128), u32),
            pltpu.VMEM((S, D), bf16),
            pltpu.VMEM((S, D), f32),
            pltpu.VMEM((S, D), f32),
            pltpu.VMEM((_PRE, D), f32),
            pltpu.VMEM((S, D), bf16),
            pltpu.VMEM((H, 8, 128), f32),
            pltpu.VMEM((H, 8, 128), f32),
            pltpu.VMEM((H, 8, 128), f32),
            pltpu.VMEM((H, 8, 128), f32),
            pltpu.VMEM((16, H * Dh), u32),
            pltpu.VMEM((24, H * Dh), u32),
            pltpu.VMEM((H // 2, 40, 128), u32),
            pltpu.VMEM((H // 2, 40, 128), u32),
            pltpu.VMEM((H // 2, 40, 128), u32),
            pltpu.VMEM((24, D), u32),
            pltpu.VMEM(((S - _PRE) // (S // (2 * SEG)) // 2, D), u32),
            pltpu.VMEM(((S - _PRE) // (S // (2 * SEG)) // 2, F), u32),
            pltpu.VMEM((_PRE // 2, D), u32),
            pltpu.VMEM((_PRE // 2, _FCH), u32),
            pltpu.SemaphoreType.DMA((S // _XCH,)),
            pltpu.SemaphoreType.DMA((_FCH // 128,)),
            pltpu.SemaphoreType.DMA((2 * (F // _FCH),)),
            pltpu.SemaphoreType.DMA((3,)),
            pltpu.SemaphoreType.DMA((1,)),
            pltpu.SemaphoreType.DMA((1,)),
        ],
        compiler_params=pltpu.CompilerParams(
            vmem_limit_bytes=124 * 1024 * 1024,
            flags={"XLA_TPU_EVENLY_DISTRIBUTE_CRITICAL_NODES": True}),
    )(mem0, x, A_Wq, A_Wk, A_Wv, wo, B_w_gate, B_w_up, B_w_down)
    return out.reshape(B, S, D)
```

```python
import functools

import jax
import jax.numpy as jnp
import jax.experimental.pallas as pl
import jax.experimental.pallas.tpu as pltpu

_PRE = 1024
_FCH = 512
_GRP = 8
_SLOTS = [4,2,2,2,2,2,2,2,2,2,2, 2,2,1,1,1,1,1,1,1,1,0]
_XCH = 256


def _sigmoid(x):
    return 1.0 / (1.0 + jnp.exp(-x))


def _bf16(x):
    return x.astype(jnp.bfloat16)


def _w(ref_val):
    return pltpu.bitcast(ref_val, jnp.bfloat16)


def _p(val):
    return pltpu.bitcast(val, jnp.uint32)


def _dot(a, b):
    return jnp.dot(a, b, preferred_element_type=jnp.float32)


def _kernel(mem0_ref, x_hbm, wq_hbm, wk_hbm, wv_hbm, wo_hbm, wg_hbm, wu_hbm, wd_hbm,
            out_hbm,
            wqkv, wo, wg, wu, wd, stg, x_scr, xn_scr, g_scr, acc_scr, out_scr,
            cq, ck, cv, co, oa, ob, q_s, k_s, v_s, lhs_s, xg_s, h_s, xb_s, hp_s,
            sem_x, sem_u0, sem_glu, sem_qkv, sem_o, sem_out,
            *, S, D, H, M, SEG, F):
    NF = F // 128
    ND = D // 128
    NCH = F // _FCH
    TPC = _FCH // 128
    NXC = S // _XCH
    scale = 128 ** (-0.5)

    def x_copy(i):
        return pltpu.make_async_copy(x_hbm.at[pl.ds(i * _XCH, _XCH), :], x_scr.at[pl.ds(i * _XCH, _XCH), :],
                                     sem_x.at[i])

    def up_copies(f):
        cps = []
        for j in range(TPC):
            c = f * TPC + j
            cps.append(pltpu.make_async_copy(
                wg_hbm.at[:, pl.ds(c * 128, 128)], wg.at[c].bitcast(jnp.bfloat16), sem_glu.at[f]))
            cps.append(pltpu.make_async_copy(
                wu_hbm.at[:, pl.ds(c * 128, 128)], wu.at[c].bitcast(jnp.bfloat16), sem_glu.at[f]))
        return cps

    def down_copies(f):
        return [pltpu.make_async_copy(
            wd_hbm.at[pl.ds(f * _FCH, _FCH), pl.ds(n * 128, 128)],
            wd.at[n, pl.ds(f * (_FCH // 2), _FCH // 2), :].bitcast(jnp.bfloat16), sem_glu.at[NCH + f])
            for n in range(ND)]

    def qkv_copies(i):
        w32 = (wq_hbm, wk_hbm, wv_hbm)[i].bitcast(jnp.uint32)
        return [pltpu.make_async_copy(w32.at[:, j, :], stg.at[i, j], sem_qkv.at[i]) for j in range(H // 2)]

    def o_copies():
        return [pltpu.make_async_copy(wo_hbm.at[:, pl.ds(n * 128, 128)],
                                      wo.at[n].bitcast(jnp.bfloat16), sem_o.at[0]) for n in range(ND)]

    def out_copy(r0, rows):
        return pltpu.make_async_copy(out_scr.at[pl.ds(r0, rows), :], out_hbm.at[pl.ds(r0, rows), :], sem_out.at[0])

    def layernorm(i):
        for r in range(i * _XCH, (i + 1) * _XCH, 128):
            x = x_scr[r:r + 128, :].astype(jnp.float32)
            m = jnp.mean(x, axis=-1, keepdims=True)
            xc = x - m
            v = jnp.mean(xc * xc, axis=-1, keepdims=True)
            xn_scr[r:r + 128, :] = xc / jnp.sqrt(v + 1e-05)

    def convert(i):
        for gi in range(D // 16):
            for j in range(H // 2):
                a = stg[i, j, pl.ds(gi * 16, 8, stride=2), :]
                b = stg[i, j, pl.ds(gi * 16 + 1, 8, stride=2), :]
                wqkv[i * H + 2 * j, gi * 8:gi * 8 + 8, :] = (a & jnp.uint32(0xFFFF)) | (b << 16)
                wqkv[i * H + 2 * j + 1, gi * 8:gi * 8 + 8, :] = (a >> 16) | (b & jnp.uint32(0xFFFF0000))

    NPX = _PRE // _XCH

    def up0(j):
        return [pltpu.make_async_copy(wg_hbm.at[:, pl.ds(j * 128, 128)], wg.at[j].bitcast(jnp.bfloat16), sem_u0.at[j]),
                pltpu.make_async_copy(wu_hbm.at[:, pl.ds(j * 128, 128)], wu.at[j].bitcast(jnp.bfloat16), sem_u0.at[j])]

    def up_tile(c, j, m0, mb):
        xb = _w(xb_s[m0 // 2:(m0 + mb) // 2, :])
        g = _dot(xb, _w(wg[c]))
        u = _dot(xb, _w(wu[c]))
        hp_s[m0 // 2:(m0 + mb) // 2, j * 128:(j + 1) * 128] = _p(_bf16(_sigmoid(g) * u))

    x_copy(0).start()
    for c in up0(0):
        c.start()
    for i in range(1, NPX):
        x_copy(i).start()
    for i in range(NPX):
        x_copy(i).wait()
        if i + 1 < TPC:
            for c in up0(i + 1):
                c.start()
        if i == NPX - 1:
            for c in down_copies(0):
                c.start()
        layernorm(i)
        xb_s[i * (_XCH // 2):(i + 1) * (_XCH // 2), :] = _p(_bf16(xn_scr[i * _XCH:(i + 1) * _XCH, :]))
        if i == 0:
            for c in up0(0):
                c.wait()
        up_tile(0, 0, i * _XCH, _XCH)

    for f in range(NCH):
        if f == 0:
            for j in range(1, TPC):
                for c in up0(j):
                    c.wait()
                if j == 1:
                    for c in up_copies(1) + down_copies(1):
                        c.start()
                up_tile(j, j, 0, _PRE)
        else:
            for c in up_copies(f) + down_copies(f):
                c.wait()
        if f + 2 < NCH:
            for c in up_copies(f + 2) + down_copies(f + 2):
                c.start()
        if f < 3:
            for c in qkv_copies(f):
                c.start()
        if f == 3:
            for c in o_copies():
                c.start()
            for i in range(NPX, NXC):
                x_copy(i).start()
        if f >= NCH - 3:
            i = f - (NCH - 3)
            for c in qkv_copies(i):
                c.wait()
        if f == NCH - 1:
            for i in range(NPX, NXC):
                x_copy(i).wait()
        if f > 0:
            for j in range(TPC):
                up_tile(f * TPC + j, j, 0, _PRE)
        if f >= NCH - 3:
            convert(f - (NCH - 3))
        if f == NCH - 1:
            for i in range(NPX, NXC):
                layernorm(i)
        if f == 0:
            for c in down_copies(f):
                c.wait()
        for m0 in range(0, _PRE, _XCH):
          ms = slice(m0, m0 + _XCH)
          for n in range(ND):
            y = _dot(_w(hp_s[m0 // 2:(m0 + _XCH) // 2, :]), _w(wd[n, f * (_FCH // 2):(f + 1) * (_FCH // 2), :]))
            if f == 0:
                acc_scr[ms, n * 128:(n + 1) * 128] = y
            elif f < NCH - 1:
                acc_scr[ms, n * 128:(n + 1) * 128] += y
            else:
                y = acc_scr[ms, n * 128:(n + 1) * 128] + y
                g_scr[ms, n * 128:(n + 1) * 128] = y * _sigmoid(y)
    for c in o_copies():
        c.wait()

    L = M + SEG
    L2 = 2 * L
    row = jax.lax.broadcasted_iota(jnp.int32, (L2, L2), 0)
    col = jax.lax.broadcasted_iota(jnp.int32, (L2, L2), 1)
    rm = jnp.where(row >= L, row - L, row)
    cm = jnp.where(col >= L, col - L, col)
    mask = ((row >= L) == (col >= L)) & ((rm < M) | (rm >= cm))
    G = _GRP // 2
    NG = H // 2 // G
    maskg = jnp.concatenate([mask] * G, axis=0)

    def attn_group(p0, fillers):
        ss = []
        for pp in range(p0, p0 + G):
            ss.append(jax.lax.dot_general(_w(q_s[pp]), _w(k_s[pp]), (((1,), (1,)), ((), ())),
                                          preferred_element_type=jnp.float32))
        fillers()
        s = jnp.concatenate(ss, axis=0) * scale
        s = jnp.where(maskg, s, -1000000000.0)
        m = jnp.max(s, axis=-1, keepdims=True)
        e = jnp.exp(s - m)
        p = _bf16(e / jnp.sum(e, axis=-1, keepdims=True))
        fillers()
        outs = []
        for i in range(G):
            o = _dot(p[i * L2:(i + 1) * L2], _w(v_s[p0 + i]))
            outs += [o[0:L], o[L:L2]]
        return outs

    NIT = S // (2 * SEG)
    GT = (S - _PRE) // NIT

    def pair(t, mem):
        r0 = pl.multiple_of(t * (2 * SEG), 2 * SEG)
        rg = pl.multiple_of(_PRE + t * GT, 8)
        xg_s[...] = _p(_bf16(xn_scr[pl.ds(rg, GT), :]))

        def glu_up(c):
            g = _dot(_w(xg_s[...]), _w(wg[c]))
            u = _dot(_w(xg_s[...]), _w(wu[c]))
            h_s[:, c * 128:(c + 1) * 128] = _p(_bf16(_sigmoid(g) * u))

        def glu_down(n):
            y = _dot(_w(h_s[...]), _w(wd[n]))
            g_scr[pl.ds(rg, GT), n * 128:(n + 1) * 128] = y * _sigmoid(y)

        tasks = [functools.partial(glu_up, c) for c in range(NF)] + [functools.partial(glu_down, n) for n in range(ND)]
        counts = list(_SLOTS)
        assert sum(counts) == len(tasks), (sum(counts), len(tasks))
        state = {"slot": 0, "done": 0}

        def fill():
            for _ in range(counts[state["slot"]]):
                tasks[state["done"]]()
                state["done"] += 1
            state["slot"] += 1

        lhs_s[...] = _p(_bf16(jnp.concatenate([mem, xn_scr[pl.ds(r0, 40), :]], axis=0)))
        fill()
        for pp in range(H // 2):
            for i, (dst, c_) in enumerate(((q_s, cq), (k_s, ck), (v_s, cv))):
                ys = []
                for hh in (2 * pp, 2 * pp + 1):
                    y = _dot(_w(lhs_s[...]), _w(wqkv[i * H + hh]))
                    c_[hh] = y[L:L + 8]
                    ys.append(y[0:L])
                dst[pp] = _p(_bf16(jnp.concatenate(ys, axis=0)))
        fill()
        for gi in range(NG):
            os_ = attn_group(gi * G, fill)
            for i, o in enumerate(os_):
                hh = gi * G * 2 + i
                oa[:, hh * 128:(hh + 1) * 128] = _p(_bf16(o[0:32]))
                co[hh] = o[32:40]
        fill()
        ya = jnp.concatenate([_dot(_w(oa[...]), _w(wo[n])) for n in range(ND)], axis=1)
        mem = ya[0:M]
        lhs_s[0:16, :] = _p(_bf16(jnp.concatenate([mem, xn_scr[pl.ds(r0 + 40, 24), :]], axis=0)))
        fill()
        for pp in range(H // 2):
            for i, (dst, c_) in enumerate(((q_s, cq), (k_s, ck), (v_s, cv))):
                ys = []
                for hh in (2 * pp, 2 * pp + 1):
                    y = _dot(_w(lhs_s[0:16, :]), _w(wqkv[i * H + hh]))
                    ys += [y[0:8], c_[hh], y[8:32]]
                dst[pp] = _p(_bf16(jnp.concatenate(ys, axis=0)))
        fill()
        for gi in range(NG):
            os_ = attn_group(gi * G, fill)
            for i, o in enumerate(os_):
                hh = gi * G * 2 + i
                ob[:, hh * 128:(hh + 1) * 128] = _p(_bf16(jnp.concatenate([o[0:8], co[hh], o[8:40]], axis=0)))
        fill()
        yb = jnp.concatenate([_dot(_w(ob[...]), _w(wo[n])) for n in range(ND)], axis=1)
        mem = yb[0:M]
        s = jnp.concatenate([ya[8:32], yb[8:48]], axis=0)
        x = x_scr[pl.ds(r0, 2 * SEG), :].astype(jnp.float32)
        out_scr[pl.ds(r0, 2 * SEG), :] = (x + s * g_scr[pl.ds(r0, 2 * SEG), :]).astype(out_scr.dtype)
        out_copy(r0, 2 * SEG).start()
        return mem

    jax.lax.fori_loop(0, NIT, pair, mem0_ref[...].astype(jnp.float32))
    for t in range(NIT):
        out_copy(t * 2 * SEG, 2 * SEG).wait()


@functools.partial(jax.jit, static_argnames=("A_seg_len",))
def pallas_recurrent_scan__memory_aug_recurrent_mem_tr__glu_gated_glu__prompt_kernel(
    A_x, A_mem0, A_Wq, A_Wk, A_Wv, A_Wo, A_seg_len, B_x, B_w_gate, B_w_up, B_w_down,
):
    del B_x
    B, S, D = A_x.shape
    H, Dh = A_Wq.shape[1], A_Wq.shape[2]
    M = A_mem0.shape[1]
    SEG = A_seg_len
    F = B_w_gate.shape[1]
    assert B == 1 and Dh == 128 and M == 8 and SEG == 32
    x = A_x.reshape(S, D)
    mem0 = A_mem0.reshape(M, D)
    wo = A_Wo.reshape(H * Dh, D)
    u32, f32, bf16 = jnp.uint32, jnp.float32, jnp.bfloat16
    anyspec = pl.BlockSpec(memory_space=pl.ANY)
    out = pl.pallas_call(
        functools.partial(_kernel, S=S, D=D, H=H, M=M, SEG=SEG, F=F),
        out_shape=jax.ShapeDtypeStruct((S, D), A_x.dtype),
        in_specs=[pl.BlockSpec(memory_space=pltpu.VMEM)] + [anyspec] * 8,
        out_specs=anyspec,
        scratch_shapes=[
            pltpu.VMEM((3 * H, D // 2, 128), u32),
            pltpu.VMEM((D // 128, H * Dh // 2, 128), u32),
            pltpu.VMEM((F // 128, D // 2, 128), u32),
            pltpu.VMEM((F // 128, D // 2, 128), u32),
            pltpu.VMEM((D // 128, F // 2, 128), u32),
            pltpu.VMEM((3, H // 2, D, 128), u32),
            pltpu.VMEM((S, D), bf16),
            pltpu.VMEM((S, D), f32),
            pltpu.VMEM((S, D), f32),
            pltpu.VMEM((_PRE, D), f32),
            pltpu.VMEM((S, D), bf16),
            pltpu.VMEM((H, 8, 128), f32),
            pltpu.VMEM((H, 8, 128), f32),
            pltpu.VMEM((H, 8, 128), f32),
            pltpu.VMEM((H, 8, 128), f32),
            pltpu.VMEM((16, H * Dh), u32),
            pltpu.VMEM((24, H * Dh), u32),
            pltpu.VMEM((H // 2, 40, 128), u32),
            pltpu.VMEM((H // 2, 40, 128), u32),
            pltpu.VMEM((H // 2, 40, 128), u32),
            pltpu.VMEM((24, D), u32),
            pltpu.VMEM(((S - _PRE) // (S // (2 * SEG)) // 2, D), u32),
            pltpu.VMEM(((S - _PRE) // (S // (2 * SEG)) // 2, F), u32),
            pltpu.VMEM((_PRE // 2, D), u32),
            pltpu.VMEM((_PRE // 2, _FCH), u32),
            pltpu.SemaphoreType.DMA((S // _XCH,)),
            pltpu.SemaphoreType.DMA((_FCH // 128,)),
            pltpu.SemaphoreType.DMA((2 * (F // _FCH),)),
            pltpu.SemaphoreType.DMA((3,)),
            pltpu.SemaphoreType.DMA((1,)),
            pltpu.SemaphoreType.DMA((1,)),
        ],
        compiler_params=pltpu.CompilerParams(
            vmem_limit_bytes=124 * 1024 * 1024,
            flags={"XLA_TPU_EVENLY_DISTRIBUTE_CRITICAL_NODES": True}),
    )(mem0, x, A_Wq, A_Wk, A_Wv, wo, B_w_gate, B_w_up, B_w_down)
    return out.reshape(B, S, D)
```
